```python
import jax
import jax.numpy as jnp

def _softmax(x, axis=-1):
    return jax.nn.softmax(x, axis=axis)

def _gelu(x):
    return jax.nn.gelu(x, approximate=True)

def _silu(x):
    return jax.nn.silu(x)

def _sigmoid(x):
    return jax.nn.sigmoid(x)

def _layernorm(x, axis=-1, eps=1e-05):
    m = jnp.mean(x, axis=axis, keepdims=True)
    v = jnp.var(x, axis=axis, keepdims=True)
    return (x - m) / jnp.sqrt(v + eps)

def _scatter_add(tgt, idx, src, axis=0):
    return tgt.at[idx].add(src)

def _segment_sum(src, seg, n):
    return jax.ops.segment_sum(src, seg, n)

class _Rng:

    def __init__(self, key):
        self._k = key

    def _next(self):
        self._k, sub = jax.random.split(self._k)
        return sub

    def normal(self, shape):
        return jax.random.normal(self._next(), shape, dtype=jnp.bfloat16)

    def randint(self, lo, hi, shape):
        return jax.random.randint(self._next(), shape, lo, hi, dtype=jnp.int32)

    def uniform(self, shape, lo=0.0, hi=1.0):
        return jax.random.uniform(self._next(), shape, jnp.bfloat16, lo, hi)

    def permutation(self, n):
        return jax.random.permutation(self._next(), n)
kernel_name = 'adaLN_cond__memory_aug_recurrent_mem_tr__moe_arch_mod__prompt'

def setup_inputs():
    _rng = _Rng(jax.random.key(int.from_bytes(__import__("os").urandom(4), "little")))
    _w = lambda a: (lambda t: t.astype(jnp.bfloat16) if jnp.issubdtype(t.dtype, jnp.floating) else t)(jnp.asarray(a))

    def _A_setup():
        B, S, Dm = (1, 2048, 1024)
        H, Dh = (32, 128)
        M, seg = (8, 32)
        seg = min(seg, S)
        S = S // seg * seg
        return {'x': _w((lambda *s: _rng.normal(s) * 0.05)(B, S, Dm)), 'mem0': _w((lambda *s: _rng.normal(s) * 0.05)(B, M, Dm)), 'Wq': _w((lambda *s: _rng.normal(s) * 0.05)(Dm, H, Dh) * Dm ** (-0.5)), 'Wk': _w((lambda *s: _rng.normal(s) * 0.05)(Dm, H, Dh) * Dm ** (-0.5)), 'Wv': _w((lambda *s: _rng.normal(s) * 0.05)(Dm, H, Dh) * Dm ** (-0.5)), 'Wo': _w((lambda *s: _rng.normal(s) * 0.05)(H, Dh, Dm) * (H * Dh) ** (-0.5)), 'seg_len': seg}
    _A_in = _A_setup()

    def _B_setup():
        B, S, D, F, C = (1, 2048, 1024, 3584, 2)
        return {'x': _w((lambda *s: _rng.normal(s) * 0.05)(B, S, D)), 'w_r': _w((lambda *s: _rng.normal(s) * 0.05)(D)), 'w_gate': _w((lambda *s: _rng.normal(s) * 0.05)(D, F)), 'w_up': _w((lambda *s: _rng.normal(s) * 0.05)(D, F)), 'w_down': _w((lambda *s: _rng.normal(s) * 0.05)(F, D))}
    _B_in = _B_setup()
    return {'A_x': _A_in['x'], 'A_mem0': _A_in['mem0'], 'A_Wq': _A_in['Wq'], 'A_Wk': _A_in['Wk'], 'A_Wv': _A_in['Wv'], 'A_Wo': _A_in['Wo'], 'A_seg_len': _A_in['seg_len'], 'B_x': _B_in['x'], 'B_w_r': _B_in['w_r'], 'B_w_gate': _B_in['w_gate'], 'B_w_up': _B_in['w_up'], 'B_w_down': _B_in['w_down'], 'c': _w((lambda *s: _rng.normal(s) * 0.05)(1, 1024)), 'w_mod': _w((lambda *s: _rng.normal(s) * 0.05)(1024, 6 * 1024) * 1024 ** (-0.5))}

def reference(A_x, A_mem0, A_Wq, A_Wk, A_Wv, A_Wo, A_seg_len, B_x, B_w_r, B_w_gate, B_w_up, B_w_down, c, w_mod):

    def _A_ref(x, mem0, Wq, Wk, Wv, Wo, seg_len):
        B, S, Dm = x.shape
        H, Dh = (Wq.shape[1], Wq.shape[2])
        M = mem0.shape[1]
        scale = Dh ** (-0.5)
        n_seg = S // seg_len
        L = M + seg_len
        idx = jnp.arange(L)
        mask = (idx[:, None] < M) | (idx[:, None] >= idx[None, :])
        mem = mem0
        outs = []
        for s in range(n_seg):
            xs = x[:, s * seg_len:(s + 1) * seg_len, :].copy()
            h = jnp.concatenate([mem, xs], axis=1)
            q = jnp.einsum('btd,dhe->bhte', h, Wq)
            k = jnp.einsum('btd,dhe->bhte', h, Wk)
            v = jnp.einsum('btd,dhe->bhte', h, Wv)
            scores = jnp.einsum('bhqe,bhke->bhqk', q, k) * scale
            scores = jnp.where(mask[None, None], scores, -1000000000.0)
            p = _softmax(scores, axis=-1)
            o = jnp.einsum('bhqk,bhke->bhqe', p, v)
            o = jnp.einsum('bhte,hed->btd', o, Wo)
            mem = o[:, :M, :].copy()
            outs.append(o[:, M:, :])
        return jnp.concatenate(outs, axis=1)

    def _B_ref(x, w_r, w_gate, w_up, w_down):
        B, S, D = x.shape
        C = 2
        r = x @ w_r
        idx = jnp.argsort(-r, axis=-1)[:, :C]
        idx_e = jnp.repeat(idx.reshape(B, C, 1), D, axis=2)
        x_sel = jnp.take_along_axis(x, idx_e, axis=1)
        g = _silu(x_sel @ w_gate)
        u = x_sel @ w_up
        y = g * u @ w_down
        r_sel = _sigmoid(jnp.take_along_axis(r, idx, axis=1))
        y = y * r_sel.reshape(B, C, 1)
        b_off = (jnp.arange(B) * S).reshape(B, 1)
        flat_idx = (idx + b_off).reshape(B * C)
        zero = (x * 0.0).reshape(B * S, D)
        upd = _scatter_add(zero, flat_idx, y.reshape(B * C, D), axis=0)
        return x + upd.reshape(B, S, D)
    x = A_x
    mod = (_silu(c) @ w_mod).reshape(c.shape[0], 6, 1, -1)
    sa, ca, ga, sb, cb, gb = (mod[:, 0].copy(), mod[:, 1].copy(), mod[:, 2].copy(), mod[:, 3].copy(), mod[:, 4].copy(), mod[:, 5].copy())
    h = _layernorm(x, axis=-1) * (1 + ca) + sa
    x = x + ga * _A_ref(h, A_mem0, A_Wq, A_Wk, A_Wv, A_Wo, A_seg_len)
    h = _layernorm(x, axis=-1) * (1 + cb) + sb
    x = x + gb * _B_ref(h, B_w_r, B_w_gate, B_w_up, B_w_down)
    return x
```

```python
import functools

import jax
import jax.numpy as jnp
from jax import lax
import jax.experimental.pallas as pl
import jax.experimental.pallas.tpu as pltpu

F32 = jnp.float32
BF16 = jnp.bfloat16
EPS = 1e-05


def _dot(a, b):
    return lax.dot_general(a, b, (((1,), (0,)), ((), ())), preferred_element_type=F32)


def _dot_nt(a, b):
    return lax.dot_general(a, b, (((1,), (1,)), ((), ())), preferred_element_type=F32)


def _ln(x):
    m = jnp.mean(x, axis=-1, keepdims=True)
    d = x - m
    v = jnp.mean(d * d, axis=-1, keepdims=True)
    return d / jnp.sqrt(v + EPS)


def _rnd(x):
    return x.astype(BF16).astype(F32)


def _kernel(x_hbm, mem0_ref, wq_hbm, wk_hbm, wv_hbm, wo_hbm, wr_ref, wg_hbm, wu_hbm,
            wd_hbm, c_ref, wmod_hbm, out_hbm,
            xb, wmod_v, stage, wq_p, wk_p, wv_p, wo_v, wg_v, wu_v, wd_v,
            mem_s, r_s, mod_s, ob,
            sem_x, sem_mod, sem_stage, sem_wo, sem_ffn, sem_out,
            *, S, D, H, Dh, M, SEG, F):
    NSEG = S // SEG
    L = M + SEG
    DCH = 128
    NCH = D // DCH

    cp_mod0 = pltpu.make_async_copy(wmod_hbm.at[:, pl.ds(0, 2 * D)], wmod_v.at[:, pl.ds(0, 2 * D)], sem_mod.at[0])
    cp_mod1 = pltpu.make_async_copy(wmod_hbm.at[:, pl.ds(2 * D, 4 * D)], wmod_v.at[:, pl.ds(2 * D, 4 * D)], sem_mod.at[1])
    cp_x = pltpu.make_async_copy(x_hbm, xb, sem_x)
    cp_wo = pltpu.make_async_copy(wo_hbm, wo_v, sem_wo)
    srcs = (wq_hbm, wk_hbm, wv_hbm)
    dsts = (wq_p, wk_p, wv_p)

    def stage_cp(t, c):
        n = t * NCH + c
        return pltpu.make_async_copy(srcs[t].at[pl.ds(c * DCH, DCH)], stage.at[n], sem_stage.at[n])

    cp_mod0.start()
    cp_x.start()
    for t in range(3):
        for c in range(NCH):
            stage_cp(t, c).start()
    cp_wo.start()
    cp_mod1.start()
    cp_g = pltpu.make_async_copy(wg_hbm, wg_v, sem_ffn.at[0])
    cp_u = pltpu.make_async_copy(wu_hbm, wu_v, sem_ffn.at[1])
    cp_d = pltpu.make_async_copy(wd_hbm, wd_v, sem_ffn.at[2])
    cp_g.start()
    cp_u.start()
    cp_d.start()

    cv = jnp.broadcast_to(c_ref[...].astype(F32), (8, D))
    sc = _rnd(cv * jax.nn.sigmoid(cv))
    cp_mod0.wait()
    m0 = _rnd(_dot(sc, wmod_v[:, 0:2 * D]))
    mod_s[:, 0:2 * D] = m0
    cp_x.wait()

    for t in range(3):
        for c in range(NCH):
            stage_cp(t, c).wait()
            dsts[t][:, c * DCH:(c + 1) * DCH, :] = jnp.swapaxes(stage[t * NCH + c], 0, 1)
    cp_wo.wait()
    cp_mod1.wait()
    mod_s[:, 2 * D:6 * D] = _rnd(_dot(sc, wmod_v[:, 2 * D:6 * D]))

    mem_s[...] = mem0_ref[...].astype(F32)

    qi = lax.broadcasted_iota(jnp.int32, (L, L), 0)
    ki = lax.broadcasted_iota(jnp.int32, (L, L), 1)
    mask = (qi < M) | (qi >= ki)
    scale = Dh ** (-0.5)
    wr = wr_ref[...].astype(F32)

    def step(s, carry):
        r0 = pl.multiple_of(s * SEG, SEG)
        sa = mod_s[0:1, 0:D]
        ca = mod_s[0:1, D:2 * D]
        ga = mod_s[0:1, 2 * D:3 * D]
        sb = mod_s[0:1, 3 * D:4 * D]
        cb = mod_s[0:1, 4 * D:5 * D]
        gb = mod_s[0:1, 5 * D:6 * D]
        xs = xb[pl.ds(r0, SEG), :].astype(F32)
        hx = _rnd(_ln(xs) * (1.0 + ca) + sa)
        h = jnp.concatenate([mem_s[...], hx], axis=0)
        acc = None
        for hd in range(H):
            q = _dot(h, wq_p[hd])
            k = _dot(h, wk_p[hd]).astype(BF16)
            v = _dot(h, wv_p[hd]).astype(BF16)
            sco = _dot_nt(q, k) * scale
            sco = jnp.where(mask, sco, -1e9)
            mx = jnp.max(sco, axis=-1, keepdims=True)
            e = jnp.exp(sco - mx)
            p = e / jnp.sum(e, axis=-1, keepdims=True)
            o = _dot(p, v)
            y = _dot(o, wo_v[hd])
            acc = y if acc is None else acc + y
        acc = _rnd(acc)
        mem_s[...] = acc[0:M]
        x1 = _rnd(xs + _rnd(ga * acc[M:L]))
        h2 = _rnd(_ln(x1) * (1.0 + cb) + sb)
        r = jnp.sum(h2 * wr, axis=-1, keepdims=True)
        r_s[pl.ds(r0, SEG), :] = jnp.broadcast_to(r, (SEG, 128))
        xb[pl.ds(r0, SEG), :] = x1.astype(BF16)
        ob[pl.ds(r0, SEG), :] = (x1 + _rnd(gb * h2)).astype(BF16)
        return carry

    lax.fori_loop(0, NSEG, step, 0)

    sb = mod_s[0:1, 3 * D:4 * D]
    cb = mod_s[0:1, 4 * D:5 * D]
    gb = mod_s[0:1, 5 * D:6 * D]
    rr = _rnd(r_s[...])
    ids = lax.broadcasted_iota(jnp.int32, (S, 128), 0)
    m1 = jnp.max(rr)
    i1 = jnp.min(jnp.where(rr == m1, ids, S))
    rr2 = jnp.where(ids == i1, -jnp.inf, rr)
    m2 = jnp.max(rr2)
    i2 = jnp.min(jnp.where((rr2 == m2) & (ids != i1), ids, S))
    i1 = jnp.clip(i1, 0, S - 1)
    i2 = jnp.clip(i2, 0, S - 1)

    def load_blk(i):
        b0 = pl.multiple_of((i // 16) * 16, 16)
        x1 = xb[pl.ds(b0, 16), :].astype(F32)
        h2 = _rnd(_ln(x1) * (1.0 + cb) + sb)
        sel = lax.broadcasted_iota(jnp.int32, (16, D), 0) == (i - b0)
        return b0, x1, h2, sel

    b1, x1a, h2a, sela = load_blk(i1)
    b2, x1b, h2b, selb = load_blk(i2)
    rowa = jnp.sum(jnp.where(sela, h2a, 0.0), axis=0, keepdims=True)
    rowb = jnp.sum(jnp.where(selb, h2b, 0.0), axis=0, keepdims=True)
    rid = lax.broadcasted_iota(jnp.int32, (8, D), 0)
    xsel = jnp.where(rid == 0, rowa, jnp.where(rid == 1, rowb, 0.0))
    cp_g.wait()
    cp_u.wait()
    cp_d.wait()
    g = _rnd(_dot(xsel, wg_v[...]))
    g = _rnd(g * jax.nn.sigmoid(g))
    u = _rnd(_dot(xsel, wu_v[...]))
    y = _rnd(_dot(_rnd(g * u), wd_v[...]))
    s1 = _rnd(jax.nn.sigmoid(jnp.full((1, D), m1, F32)))
    s2 = _rnd(jax.nn.sigmoid(jnp.full((1, D), m2, F32)))
    ya = _rnd(y[0:1] * s1)
    yb = _rnd(y[1:2] * s2)
    selb_in_a = lax.broadcasted_iota(jnp.int32, (16, D), 0) == (i2 - b1)
    sela_in_b = lax.broadcasted_iota(jnp.int32, (16, D), 0) == (i1 - b2)
    upa = jnp.where(sela, ya, 0.0) + jnp.where(selb_in_a, yb, 0.0)
    upb = jnp.where(selb, yb, 0.0) + jnp.where(sela_in_b, ya, 0.0)
    ob[pl.ds(b1, 16), :] = (x1a + _rnd(gb * _rnd(h2a + upa))).astype(BF16)
    ob[pl.ds(b2, 16), :] = (x1b + _rnd(gb * _rnd(h2b + upb))).astype(BF16)
    cp_o = pltpu.make_async_copy(ob, out_hbm, sem_out)
    cp_o.start()
    cp_o.wait()


@functools.partial(jax.jit, static_argnames=("A_seg_len",))
def pallas_adaLN_cond__memory_aug_recurrent_mem_tr__moe_arch_mod__prompt_kernel(
    A_x, A_mem0, A_Wq, A_Wk, A_Wv, A_Wo, A_seg_len, B_x, B_w_r, B_w_gate, B_w_up,
    B_w_down, c, w_mod,
):
    del B_x
    B, S, D = A_x.shape
    assert B == 1
    M = A_mem0.shape[1]
    H, Dh = A_Wq.shape[1], A_Wq.shape[2]
    SEG = int(A_seg_len)
    F = B_w_gate.shape[1]
    NCH = D // 128
    hbm = pl.BlockSpec(memory_space=pl.ANY)
    vm = pl.BlockSpec(memory_space=pltpu.VMEM)
    scratch = [
        pltpu.VMEM((S, D), BF16),
        pltpu.VMEM((D, 6 * D), BF16),
        pltpu.VMEM((3 * NCH, 128, H, Dh), BF16),
        pltpu.VMEM((H, D, Dh), BF16),
        pltpu.VMEM((H, D, Dh), BF16),
        pltpu.VMEM((H, D, Dh), BF16),
        pltpu.VMEM((H, Dh, D), BF16),
        pltpu.VMEM((D, F), BF16),
        pltpu.VMEM((D, F), BF16),
        pltpu.VMEM((F, D), BF16),
        pltpu.VMEM((M, D), F32),
        pltpu.VMEM((S, 128), F32),
        pltpu.VMEM((8, 6 * D), F32),
        pltpu.VMEM((S, D), BF16),
        pltpu.SemaphoreType.DMA,
        pltpu.SemaphoreType.DMA((2,)),
        pltpu.SemaphoreType.DMA((3 * NCH,)),
        pltpu.SemaphoreType.DMA,
        pltpu.SemaphoreType.DMA((3,)),
        pltpu.SemaphoreType.DMA,
    ]
    out = pl.pallas_call(
        functools.partial(_kernel, S=S, D=D, H=H, Dh=Dh, M=M, SEG=SEG, F=F),
        in_specs=[hbm, vm, hbm, hbm, hbm, hbm, vm, hbm, hbm, hbm, vm, hbm],
        out_specs=hbm,
        out_shape=jax.ShapeDtypeStruct((S, D), A_x.dtype),
        scratch_shapes=scratch,
        compiler_params=pltpu.CompilerParams(vmem_limit_bytes=120 * 2**20),
    )(A_x.reshape(S, D), A_mem0.reshape(M, D), A_Wq, A_Wk, A_Wv, A_Wo,
      B_w_r.reshape(1, D), B_w_gate, B_w_up, B_w_down, c, w_mod)
    return out.reshape(B, S, D)
```

```python
import functools

import jax
import jax.numpy as jnp
from jax import lax
import jax.experimental.pallas as pl
import jax.experimental.pallas.tpu as pltpu

F32 = jnp.float32
BF16 = jnp.bfloat16
EPS = 1e-05


def _dot(a, b):
    return lax.dot_general(a, b, (((1,), (0,)), ((), ())), preferred_element_type=F32)


def _dot_nt(a, b):
    return lax.dot_general(a, b, (((1,), (1,)), ((), ())), preferred_element_type=F32)


def _ln(x):
    m = jnp.mean(x, axis=-1, keepdims=True)
    d = x - m
    v = jnp.mean(d * d, axis=-1, keepdims=True)
    return d / jnp.sqrt(v + EPS)


def _rnd(x):
    return x.astype(BF16).astype(F32)


def _kernel(x_hbm, mem0_ref, wq_hbm, wk_hbm, wv_hbm, wo_hbm, wr_ref, wg_hbm, wu_hbm,
            wd_hbm, c_ref, wmod_hbm, out_hbm,
            xb, wmod_v, stage, wq_p, wk_p, wv_p, wo_v, wg_v, wu_v, wd_v,
            wo_p, h_s, a_s, o_s, x1b, r_s, mod_s, ob,
            sem_x, sem_mod, sem_stage, sem_wo, sem_ffn, sem_out,
            *, S, D, H, Dh, M, SEG, F):
    NSEG = S // SEG
    L = M + SEG
    DCH = 128
    NCH = D // DCH

    cp_mod0 = pltpu.make_async_copy(wmod_hbm.at[:, pl.ds(0, 2 * D)], wmod_v.at[:, pl.ds(0, 2 * D)], sem_mod.at[0])
    cp_mod1 = pltpu.make_async_copy(wmod_hbm.at[:, pl.ds(2 * D, 4 * D)], wmod_v.at[:, pl.ds(2 * D, 4 * D)], sem_mod.at[1])
    cp_x = pltpu.make_async_copy(x_hbm, xb, sem_x)
    cp_wo = pltpu.make_async_copy(wo_hbm, wo_v, sem_wo)
    srcs = (wq_hbm, wk_hbm, wv_hbm)
    dsts = (wq_p, wk_p, wv_p)

    def stage_cp(t, c):
        n = t * NCH + c
        return pltpu.make_async_copy(srcs[t].at[pl.ds(c * DCH, DCH)], stage.at[n], sem_stage.at[n])

    cp_mod0.start()
    cp_x.start()
    for t in range(3):
        for c in range(NCH):
            stage_cp(t, c).start()
    cp_wo.start()
    cp_mod1.start()
    cp_g = pltpu.make_async_copy(wg_hbm, wg_v, sem_ffn.at[0])
    cp_u = pltpu.make_async_copy(wu_hbm, wu_v, sem_ffn.at[1])
    cp_d = pltpu.make_async_copy(wd_hbm, wd_v, sem_ffn.at[2])
    cp_g.start()
    cp_u.start()
    cp_d.start()

    cv = jnp.broadcast_to(c_ref[...].astype(F32), (8, D))
    sc = _rnd(cv * jax.nn.sigmoid(cv))
    cp_mod0.wait()
    m0 = _rnd(_dot(sc, wmod_v[:, 0:2 * D]))
    mod_s[:, 0:2 * D] = m0
    cp_x.wait()

    for t in range(3):
        for c in range(NCH):
            stage_cp(t, c).wait()
            tr = pltpu.bitcast(jnp.swapaxes(stage[t * NCH + c], 0, 1), jnp.int32)
            for hd in range(H):
                dsts[t][hd // 4, c * DCH // 2:(c + 1) * DCH // 2, (hd % 4) * Dh:(hd % 4 + 1) * Dh] = tr[hd]
    cp_wo.wait()
    for hd in range(H):
        wo_p[hd * Dh // 2:(hd + 1) * Dh // 2, :] = pltpu.bitcast(wo_v[hd], jnp.int32)
    cp_mod1.wait()
    mod_s[:, 2 * D:6 * D] = _rnd(_dot(sc, wmod_v[:, 2 * D:6 * D]))

    h_s[0:M, :] = mem0_ref[...].astype(F32)

    qi = lax.broadcasted_iota(jnp.int32, (L, L), 0)
    ki = lax.broadcasted_iota(jnp.int32, (L, L), 1)
    mask = (qi < M) | (qi >= ki)
    scale = Dh ** (-0.5)
    wr = wr_ref[...].astype(F32)

    sa = mod_s[0:1, 0:D]
    ca = mod_s[0:1, D:2 * D]
    ga = mod_s[0:1, 2 * D:3 * D]
    sb = mod_s[0:1, 3 * D:4 * D]
    cb = mod_s[0:1, 4 * D:5 * D]
    gb = mod_s[0:1, 5 * D:6 * D]

    def pre(s):
        r0 = pl.multiple_of(s * SEG, SEG)
        xs = xb[pl.ds(r0, SEG), :].astype(F32)
        h_s[M:L, :] = _rnd(_ln(xs) * (1.0 + ca) + sa)

    def post(s):
        r0 = pl.multiple_of(s * SEG, SEG)
        xs = xb[pl.ds(r0, SEG), :].astype(F32)
        x1 = _rnd(xs + _rnd(ga * a_s[...]))
        h2 = _rnd(_ln(x1) * (1.0 + cb) + sb)
        r = jnp.sum(h2 * wr, axis=-1, keepdims=True)
        r_s[pl.ds(r0, SEG), :] = jnp.broadcast_to(r, (SEG, 128))
        x1b[pl.ds(r0, SEG), :] = x1.astype(BF16)
        ob[pl.ds(r0, SEG), :] = (x1 + _rnd(gb * h2)).astype(BF16)

    def wtile(ref, hd):
        return pltpu.bitcast(ref[hd], BF16)

    def softmax(sco):
        sco = jnp.where(mask, sco * scale, -1e9)
        mx = jnp.max(sco, axis=-1, keepdims=True)
        e = jnp.exp(sco - mx)
        return e / jnp.sum(e, axis=-1, keepdims=True)

    a_s[...] = jnp.zeros_like(a_s)
    pre(0)
    GH = 4
    NG = H // GH
    HS = H - 8

    def step(s, carry):
        h = h_s[...]
        post(jnp.maximum(s - 1, 0))
        q = k = v = None

        def qk(q, k):
            return [_dot_nt(q[:, j * Dh:(j + 1) * Dh], k[:, j * Dh:(j + 1) * Dh]) for j in range(GH)]

        def pv(sco, v, g):
            for j in range(GH):
                hd = g * GH + j
                o_s[:, hd * Dh:(hd + 1) * Dh] = _dot(softmax(sco[j]), v[:, j * Dh:(j + 1) * Dh])

        for g in range(NG):
            qn = _dot(h, wtile(wq_p, g))
            if g > 0:
                sco = qk(q, k)
            kn = _dot(h, wtile(wk_p, g)).astype(BF16)
            if g > 0:
                pv(sco, v, g - 1)
            vn = _dot(h, wtile(wv_p, g)).astype(BF16)
            q, k, v = qn, kn, vn
        sco = qk(q, k)
        acc = _dot(o_s[:, 0:HS * Dh], pltpu.bitcast(wo_p[0:HS * Dh // 2, :], BF16))
        pv(sco, v, NG - 1)
        acc = acc + _dot(o_s[:, HS * Dh:H * Dh], pltpu.bitcast(wo_p[HS * Dh // 2:H * Dh // 2, :], BF16))
        acc = _rnd(acc)
        h_s[0:M, :] = acc[0:M]
        a_s[...] = acc[M:L]
        pre(jnp.minimum(s + 1, NSEG - 1))
        return carry

    lax.fori_loop(0, NSEG, step, 0)
    post(NSEG - 1)

    rr = _rnd(r_s[...])
    ids = lax.broadcasted_iota(jnp.int32, (S, 128), 0)
    m1 = jnp.max(rr)
    i1 = jnp.min(jnp.where(rr == m1, ids, S))
    rr2 = jnp.where(ids == i1, -jnp.inf, rr)
    m2 = jnp.max(rr2)
    i2 = jnp.min(jnp.where((rr2 == m2) & (ids != i1), ids, S))
    i1 = jnp.clip(i1, 0, S - 1)
    i2 = jnp.clip(i2, 0, S - 1)

    def load_blk(i):
        b0 = pl.multiple_of((i // 16) * 16, 16)
        x1 = x1b[pl.ds(b0, 16), :].astype(F32)
        h2 = _rnd(_ln(x1) * (1.0 + cb) + sb)
        sel = lax.broadcasted_iota(jnp.int32, (16, D), 0) == (i - b0)
        return b0, x1, h2, sel

    b1, x1a, h2a, sela = load_blk(i1)
    b2, x1b, h2b, selb = load_blk(i2)
    rowa = jnp.sum(jnp.where(sela, h2a, 0.0), axis=0, keepdims=True)
    rowb = jnp.sum(jnp.where(selb, h2b, 0.0), axis=0, keepdims=True)
    rid = lax.broadcasted_iota(jnp.int32, (8, D), 0)
    xsel = jnp.where(rid == 0, rowa, jnp.where(rid == 1, rowb, 0.0))
    cp_g.wait()
    cp_u.wait()
    cp_d.wait()
    g = _rnd(_dot(xsel, wg_v[...]))
    g = _rnd(g * jax.nn.sigmoid(g))
    u = _rnd(_dot(xsel, wu_v[...]))
    y = _rnd(_dot(_rnd(g * u), wd_v[...]))
    s1 = _rnd(jax.nn.sigmoid(jnp.full((1, D), m1, F32)))
    s2 = _rnd(jax.nn.sigmoid(jnp.full((1, D), m2, F32)))
    ya = _rnd(y[0:1] * s1)
    yb = _rnd(y[1:2] * s2)
    selb_in_a = lax.broadcasted_iota(jnp.int32, (16, D), 0) == (i2 - b1)
    sela_in_b = lax.broadcasted_iota(jnp.int32, (16, D), 0) == (i1 - b2)
    upa = jnp.where(sela, ya, 0.0) + jnp.where(selb_in_a, yb, 0.0)
    upb = jnp.where(selb, yb, 0.0) + jnp.where(sela_in_b, ya, 0.0)
    ob[pl.ds(b1, 16), :] = (x1a + _rnd(gb * _rnd(h2a + upa))).astype(BF16)
    ob[pl.ds(b2, 16), :] = (x1b + _rnd(gb * _rnd(h2b + upb))).astype(BF16)
    cp_o = pltpu.make_async_copy(ob, out_hbm, sem_out)
    cp_o.start()
    cp_o.wait()


@functools.partial(jax.jit, static_argnames=("A_seg_len",))
def pallas_adaLN_cond__memory_aug_recurrent_mem_tr__moe_arch_mod__prompt_kernel(
    A_x, A_mem0, A_Wq, A_Wk, A_Wv, A_Wo, A_seg_len, B_x, B_w_r, B_w_gate, B_w_up,
    B_w_down, c, w_mod,
):
    del B_x
    B, S, D = A_x.shape
    assert B == 1
    M = A_mem0.shape[1]
    H, Dh = A_Wq.shape[1], A_Wq.shape[2]
    SEG = int(A_seg_len)
    F = B_w_gate.shape[1]
    NCH = D // 128
    hbm = pl.BlockSpec(memory_space=pl.ANY)
    vm = pl.BlockSpec(memory_space=pltpu.VMEM)
    scratch = [
        pltpu.VMEM((S, D), BF16),
        pltpu.VMEM((D, 6 * D), BF16),
        pltpu.VMEM((3 * NCH, 128, H, Dh), BF16),
        pltpu.VMEM((H // 4, D // 2, 4 * Dh), jnp.int32),
        pltpu.VMEM((H // 4, D // 2, 4 * Dh), jnp.int32),
        pltpu.VMEM((H // 4, D // 2, 4 * Dh), jnp.int32),
        pltpu.VMEM((H, Dh, D), BF16),
        pltpu.VMEM((D, F), BF16),
        pltpu.VMEM((D, F), BF16),
        pltpu.VMEM((F, D), BF16),
        pltpu.VMEM((H * Dh // 2, D), jnp.int32),
        pltpu.VMEM((M + SEG, D), F32),
        pltpu.VMEM((SEG, D), F32),
        pltpu.VMEM((M + SEG, H * Dh), F32),
        pltpu.VMEM((S, D), BF16),
        pltpu.VMEM((S, 128), F32),
        pltpu.VMEM((8, 6 * D), F32),
        pltpu.VMEM((S, D), BF16),
        pltpu.SemaphoreType.DMA,
        pltpu.SemaphoreType.DMA((2,)),
        pltpu.SemaphoreType.DMA((3 * NCH,)),
        pltpu.SemaphoreType.DMA,
        pltpu.SemaphoreType.DMA((3,)),
        pltpu.SemaphoreType.DMA,
    ]
    out = pl.pallas_call(
        functools.partial(_kernel, S=S, D=D, H=H, Dh=Dh, M=M, SEG=SEG, F=F),
        in_specs=[hbm, vm, hbm, hbm, hbm, hbm, vm, hbm, hbm, hbm, vm, hbm],
        out_specs=hbm,
        out_shape=jax.ShapeDtypeStruct((S, D), A_x.dtype),
        scratch_shapes=scratch,
        compiler_params=pltpu.CompilerParams(vmem_limit_bytes=120 * 2**20),
    )(A_x.reshape(S, D), A_mem0.reshape(M, D), A_Wq, A_Wk, A_Wv, A_Wo,
      B_w_r.reshape(1, D), B_w_gate, B_w_up, B_w_down, c, w_mod)
    return out.reshape(B, S, D)
```

```python
import functools

import jax
import jax.numpy as jnp
from jax import lax
import jax.experimental.pallas as pl
import jax.experimental.pallas.tpu as pltpu

F32 = jnp.float32
BF16 = jnp.bfloat16
EPS = 1e-05
LOG2E = 1.4426950408889634


def _dot(a, b):
    return lax.dot_general(a, b, (((1,), (0,)), ((), ())), preferred_element_type=F32)


def _dot_nt(a, b):
    return lax.dot_general(a, b, (((1,), (1,)), ((), ())), preferred_element_type=F32)


def _ln(x):
    m = jnp.mean(x, axis=-1, keepdims=True)
    d = x - m
    v = jnp.mean(d * d, axis=-1, keepdims=True)
    return d / jnp.sqrt(v + EPS)


def _rnd(x):
    return x.astype(BF16).astype(F32)


def _kernel(x_hbm, mem0_ref, wq_hbm, wk_hbm, wv_hbm, wo_hbm, wr_ref, wg_hbm, wu_hbm,
            wd_hbm, c_ref, wmod_hbm, out_hbm,
            xb, wmod_v, stage, wq_p, wk_p, wv_p, wo_v, wg_v, wu_v, wd_v,
            wo_p, h_s, o_s, a_all, r_s, mod_s, ob,
            sem_x, sem_mod, sem_stage, sem_wo, sem_ffn, sem_out, sem_patch,
            *, S, D, H, Dh, M, SEG, F):
    NSEG = S // SEG
    L = M + SEG
    DCH = 128
    NCH = D // DCH
    GH = 4
    NG = H // GH
    HS = H - 8
    NWO = 4
    WOH = H // NWO
    X0 = 4 * SEG
    OCH = 8 * SEG
    NOC = S // OCH

    cp_mod0 = pltpu.make_async_copy(wmod_hbm.at[:, pl.ds(0, 2 * D)], wmod_v.at[:, pl.ds(0, 2 * D)], sem_mod.at[0])
    cp_mod1 = pltpu.make_async_copy(wmod_hbm.at[:, pl.ds(2 * D, 4 * D)], wmod_v.at[:, pl.ds(2 * D, 4 * D)], sem_mod.at[1])
    cp_x0 = pltpu.make_async_copy(x_hbm.at[pl.ds(0, X0)], xb.at[pl.ds(0, X0)], sem_x.at[0])
    cp_x1 = pltpu.make_async_copy(x_hbm.at[pl.ds(X0, S - X0)], xb.at[pl.ds(X0, S - X0)], sem_x.at[1])
    srcs = (wq_hbm, wk_hbm, wv_hbm)
    dsts = (wq_p, wk_p, wv_p)

    def startup_cp(n):
        if n < 3 * NCH:
            t, c = divmod(n, NCH)
            return pltpu.make_async_copy(srcs[t].at[pl.ds(c * DCH, DCH)], stage.at[n], sem_stage.at[n])
        j = n - 3 * NCH
        return pltpu.make_async_copy(wo_hbm.at[pl.ds(j * WOH, WOH)], wo_v.at[pl.ds(j * WOH, WOH)], sem_wo.at[j])

    NST = 3 * NCH + NWO
    WINDOW = 4

    def ffn_cps():
        cps = []
        for j in range(F // 128):
            cps.append(pltpu.make_async_copy(wg_hbm.at[:, pl.ds(j * 128, 128)], wg_v.at[j], sem_ffn.at[0]))
            cps.append(pltpu.make_async_copy(wu_hbm.at[:, pl.ds(j * 128, 128)], wu_v.at[j], sem_ffn.at[0]))
        for j in range(D // 128):
            cps.append(pltpu.make_async_copy(wd_hbm.at[:, pl.ds(j * 128, 128)], wd_v.at[j], sem_ffn.at[0]))
        return cps

    def out_cp(j):
        return pltpu.make_async_copy(ob.at[pl.ds(j * OCH, OCH)], out_hbm.at[pl.ds(j * OCH, OCH)], sem_out.at[j])

    cp_mod0.start()
    cp_x0.start()
    for n in range(WINDOW):
        startup_cp(n).start()

    cv = jnp.broadcast_to(c_ref[...].astype(F32), (8, D))
    sc = _rnd(cv * jax.nn.sigmoid(cv))
    mod_s[:, 2 * D:6 * D] = jnp.zeros((8, 4 * D), F32)
    r_s[...] = jnp.full(r_s.shape, -jnp.inf, F32)
    h_s[0:M, :] = mem0_ref[...].astype(F32)
    cp_mod0.wait()
    mod_s[:, 0:2 * D] = _rnd(_dot(sc, wmod_v[:, 0:2 * D]))

    def staged(n):
        startup_cp(n).wait()
        if n + WINDOW < NST:
            startup_cp(n + WINDOW).start()
        elif n + WINDOW == NST:
            cp_mod1.start()
            cp_x1.start()
        if n < 3 * NCH:
            t, c = divmod(n, NCH)
            tr = pltpu.bitcast(jnp.swapaxes(stage[n], 0, 1), jnp.int32)
            for hd in range(H):
                dsts[t][hd // GH, c * DCH // 2:(c + 1) * DCH // 2, (hd % GH) * Dh:(hd % GH + 1) * Dh] = tr[hd]
        else:
            j = n - 3 * NCH
            for hd in range(j * WOH, (j + 1) * WOH):
                wo_p[hd * Dh // 2:(hd + 1) * Dh // 2, :] = pltpu.bitcast(wo_v[hd], jnp.int32)

    for n in range(3 * NCH):
        staged(n)
    cp_x0.wait()

    qi = lax.broadcasted_iota(jnp.int32, (L, L), 0)
    ki = lax.broadcasted_iota(jnp.int32, (L, L), 1)
    mask = (qi < M) | (qi >= ki)
    scale = Dh ** (-0.5)
    wr = wr_ref[...].astype(F32)

    def mods(i):
        return mod_s[0:1, i * D:(i + 1) * D]

    def pre(s):
        r0 = pl.multiple_of(s * SEG, SEG)
        xs = xb[pl.ds(r0, SEG), :].astype(F32)
        h_s[M:L, :] = _rnd(_ln(xs) * (1.0 + mods(1)) + mods(0))

    def norm2(x1):
        return _rnd(_ln(x1) * (1.0 + mods(4)) + mods(3))

    def resid(r0, n):
        xs = xb[pl.ds(r0, n), :].astype(F32)
        return _rnd(xs + _rnd(mods(2) * a_all[pl.ds(r0, n), :].astype(F32)))

    def post(s):
        r0 = pl.multiple_of(s * SEG, SEG)
        x1 = resid(r0, SEG)
        h2 = norm2(x1)
        r = jnp.sum(h2 * wr, axis=-1, keepdims=True)
        lane = lax.broadcasted_iota(jnp.int32, (SEG, 128), 1)
        r_s[...] = jnp.where(lane == s, r, r_s[...])
        ob[pl.ds(r0, SEG), :] = (x1 + _rnd(mods(5) * h2)).astype(BF16)

    def wtile(ref, g):
        return pltpu.bitcast(ref[g], BF16)

    def attend(sco, v):
        sco = jnp.where(mask, sco, -1e9 / scale)
        mx = jnp.max(sco, axis=-1, keepdims=True)
        e = jnp.exp2((sco - mx) * (scale * LOG2E))
        den = jnp.sum(e, axis=-1, keepdims=True)
        inv = pl.reciprocal(den, approx=True)
        inv = inv + inv * (1.0 - den * inv)
        return _dot(e * inv, v)

    pre(0)

    def step(s, first=False):
        h = h_s[...]
        if not first:
            post(jnp.maximum(s - 2, 0))
        q = k = v = None

        def qk(q, k):
            return [_dot_nt(q[:, j * Dh:(j + 1) * Dh], k[:, j * Dh:(j + 1) * Dh]) for j in range(GH)]

        def pv(sco, v, g):
            for j in range(GH):
                hd = g * GH + j
                o_s[:, hd * Dh:(hd + 1) * Dh] = attend(sco[j], v[:, j * Dh:(j + 1) * Dh])

        for g in range(NG):
            qn = _dot(h, wtile(wq_p, g))
            if g > 0:
                sco = qk(q, k)
            kn = _dot(h, wtile(wk_p, g)).astype(BF16)
            vn = _dot(h, wtile(wv_p, g)).astype(BF16)
            if g > 0:
                pv(sco, v, g - 1)
            q, k, v = qn, kn, vn
        sco = qk(q, k)
        if first:
            for n in range(3 * NCH, NST):
                staged(n)
        acc = _dot(o_s[:, 0:HS * Dh], pltpu.bitcast(wo_p[0:HS * Dh // 2, :], BF16))
        pv(sco, v, NG - 1)
        acc = acc + _dot(o_s[:, HS * Dh:H * Dh], pltpu.bitcast(wo_p[HS * Dh // 2:H * Dh // 2, :], BF16))
        pre(jnp.minimum(s + 1, NSEG - 1))
        acc = acc.astype(BF16)
        h_s[0:M, :] = acc[0:M].astype(F32)
        a_all[pl.ds(pl.multiple_of(s * SEG, SEG), SEG), :] = acc[M:L]
        if first:
            return

        @pl.when(s == 1)
        def _():
            cp_mod1.wait()
            cp_x1.wait()
            for cp in ffn_cps():
                cp.start()
            mod_s[:, 2 * D:6 * D] = _rnd(_dot(sc, wmod_v[:, 2 * D:6 * D]))

        @pl.when(jnp.logical_and(s > 8, s % 8 == 1))
        def _():
            j = s // 8 - 1
            r0 = pl.multiple_of(j * OCH, OCH)
            pltpu.make_async_copy(ob.at[pl.ds(r0, OCH)], out_hbm.at[pl.ds(r0, OCH)], sem_out.at[j]).start()

    step(0, first=True)
    lax.fori_loop(1, NSEG, lambda s, c: (step(s), c)[1], 0)
    post(NSEG - 2)
    post(NSEG - 1)

    rr = _rnd(r_s[...])
    ids = lax.broadcasted_iota(jnp.int32, (SEG, 128), 1) * SEG + lax.broadcasted_iota(jnp.int32, (SEG, 128), 0)
    valid = ids < S
    m1 = jnp.max(jnp.where(valid, rr, -jnp.inf))
    i1 = jnp.min(jnp.where((rr == m1) & valid, ids, S))
    rest = valid & (ids != i1)
    m2 = jnp.max(jnp.where(rest, rr, -jnp.inf))
    i2 = jnp.min(jnp.where((rr == m2) & rest, ids, S))
    i1 = jnp.clip(i1, 0, S - 1)
    i2 = jnp.clip(i2, 0, S - 1)

    row16 = lax.broadcasted_iota(jnp.int32, (16, D), 0)

    def load_blk(i):
        b0 = pl.multiple_of((i // 16) * 16, 16)
        x1 = resid(b0, 16)
        return b0, x1, norm2(x1), row16 == (i - b0)

    b1, x1a, h2a, sela = load_blk(i1)
    b2, x1c, h2c, selc = load_blk(i2)
    rowa = jnp.sum(jnp.where(sela, h2a, 0.0), axis=0, keepdims=True)
    rowc = jnp.sum(jnp.where(selc, h2c, 0.0), axis=0, keepdims=True)
    rid = lax.broadcasted_iota(jnp.int32, (8, D), 0)
    xsel = jnp.where(rid == 0, rowa, jnp.where(rid == 1, rowc, 0.0))
    for cp in ffn_cps():
        cp.wait()
    g = jnp.concatenate([_dot(xsel, wg_v[j]) for j in range(F // 128)], axis=1)
    u = jnp.concatenate([_dot(xsel, wu_v[j]) for j in range(F // 128)], axis=1)
    g = _rnd(g)
    g = _rnd(g * jax.nn.sigmoid(g))
    gu = _rnd(g * _rnd(u))
    y = _rnd(jnp.concatenate([_dot(gu, wd_v[j]) for j in range(D // 128)], axis=1))
    s1 = _rnd(jax.nn.sigmoid(jnp.full((1, D), m1, F32)))
    s2 = _rnd(jax.nn.sigmoid(jnp.full((1, D), m2, F32)))
    ya = _rnd(y[0:1] * s1)
    yc = _rnd(y[1:2] * s2)
    upa = jnp.where(sela, ya, 0.0) + jnp.where(row16 == (i2 - b1), yc, 0.0)
    upc = jnp.where(selc, yc, 0.0) + jnp.where(row16 == (i1 - b2), ya, 0.0)
    for j in range(NOC - 1):
        out_cp(j).wait()
    ob[pl.ds(b1, 16), :] = (x1a + _rnd(mods(5) * _rnd(h2a + upa))).astype(BF16)
    ob[pl.ds(b2, 16), :] = (x1c + _rnd(mods(5) * _rnd(h2c + upc))).astype(BF16)
    last0 = (NOC - 1) * OCH
    out_cp(NOC - 1).start()

    def patch_cp(b, k):
        return pltpu.make_async_copy(ob.at[pl.ds(b, 16)], out_hbm.at[pl.ds(b, 16)], sem_patch.at[k])

    send1 = b1 < last0
    send2 = jnp.logical_and(b2 < last0, b2 != b1)

    @pl.when(send1)
    def _():
        patch_cp(b1, 0).start()

    @pl.when(send2)
    def _():
        patch_cp(b2, 1).start()

    @pl.when(send1)
    def _():
        patch_cp(b1, 0).wait()

    @pl.when(send2)
    def _():
        patch_cp(b2, 1).wait()

    out_cp(NOC - 1).wait()


@functools.partial(jax.jit, static_argnames=("A_seg_len",))
def pallas_adaLN_cond__memory_aug_recurrent_mem_tr__moe_arch_mod__prompt_kernel(
    A_x, A_mem0, A_Wq, A_Wk, A_Wv, A_Wo, A_seg_len, B_x, B_w_r, B_w_gate, B_w_up,
    B_w_down, c, w_mod,
):
    del B_x
    B, S, D = A_x.shape
    assert B == 1
    M = A_mem0.shape[1]
    H, Dh = A_Wq.shape[1], A_Wq.shape[2]
    SEG = int(A_seg_len)
    F = B_w_gate.shape[1]
    NCH = D // 128
    hbm = pl.BlockSpec(memory_space=pl.ANY)
    vm = pl.BlockSpec(memory_space=pltpu.VMEM)
    scratch = [
        pltpu.VMEM((S, D), BF16),
        pltpu.VMEM((D, 6 * D), BF16),
        pltpu.VMEM((3 * NCH, 128, H, Dh), BF16),
        pltpu.VMEM((H // 4, D // 2, 4 * Dh), jnp.int32),
        pltpu.VMEM((H // 4, D // 2, 4 * Dh), jnp.int32),
        pltpu.VMEM((H // 4, D // 2, 4 * Dh), jnp.int32),
        pltpu.VMEM((H, Dh, D), BF16),
        pltpu.VMEM((F // 128, D, 128), BF16),
        pltpu.VMEM((F // 128, D, 128), BF16),
        pltpu.VMEM((D // 128, F, 128), BF16),
        pltpu.VMEM((H * Dh // 2, D), jnp.int32),
        pltpu.VMEM((M + SEG, D), F32),
        pltpu.VMEM((M + SEG, H * Dh), F32),
        pltpu.VMEM((S, D), BF16),
        pltpu.VMEM((SEG, 128), F32),
        pltpu.VMEM((8, 6 * D), F32),
        pltpu.VMEM((S, D), BF16),
        pltpu.SemaphoreType.DMA((2,)),
        pltpu.SemaphoreType.DMA((2,)),
        pltpu.SemaphoreType.DMA((3 * NCH,)),
        pltpu.SemaphoreType.DMA((4,)),
        pltpu.SemaphoreType.DMA((1,)),
        pltpu.SemaphoreType.DMA((S // (8 * SEG),)),
        pltpu.SemaphoreType.DMA((2,)),
    ]
    out = pl.pallas_call(
        functools.partial(_kernel, S=S, D=D, H=H, Dh=Dh, M=M, SEG=SEG, F=F),
        in_specs=[hbm, vm, hbm, hbm, hbm, hbm, vm, hbm, hbm, hbm, vm, hbm],
        out_specs=hbm,
        out_shape=jax.ShapeDtypeStruct((S, D), A_x.dtype),
        scratch_shapes=scratch,
        compiler_params=pltpu.CompilerParams(vmem_limit_bytes=120 * 2**20),
    )(A_x.reshape(S, D), A_mem0.reshape(M, D), A_Wq, A_Wk, A_Wv, A_Wo,
      B_w_r.reshape(1, D), B_w_gate, B_w_up, B_w_down, c, w_mod)
    return out.reshape(B, S, D)
```

```python
import functools

import jax
import jax.numpy as jnp
from jax import lax
import jax.experimental.pallas as pl
import jax.experimental.pallas.tpu as pltpu

F32 = jnp.float32
BF16 = jnp.bfloat16
EPS = 1e-05
GH = 8
HTAIL = 16
LOG2E = 1.4426950408889634


def _dot(a, b):
    return lax.dot_general(a, b, (((1,), (0,)), ((), ())), preferred_element_type=F32)


def _dot_nt(a, b):
    return lax.dot_general(a, b, (((1,), (1,)), ((), ())), preferred_element_type=F32)


def _ln(x):
    m = jnp.mean(x, axis=-1, keepdims=True)
    d = x - m
    v = jnp.mean(d * d, axis=-1, keepdims=True)
    return d / jnp.sqrt(v + EPS)


def _rnd(x):
    return x.astype(BF16).astype(F32)


def _kernel(x_hbm, mem0_ref, wq_hbm, wk_hbm, wv_hbm, wo_hbm, wr_ref, wg_hbm, wu_hbm,
            wd_hbm, c_ref, wmod_hbm, out_hbm,
            xb, wmod_v, stage, wq_p, wk_p, wv_p, wo_v, wg_v, wu_v, wd_v,
            wo_p, h_s, o_s, a_all, r_s, mod_s, ob,
            sem_x, sem_mod, sem_stage, sem_wo, sem_ffn, sem_out, sem_patch,
            *, S, D, H, Dh, M, SEG, F):
    NSEG = S // SEG
    L = M + SEG
    DCH = 128
    NCH = D // DCH
    NG = H // GH
    HS = H - HTAIL
    NWO = 4
    WOH = H // NWO
    X0 = 4 * SEG
    OCH = 8 * SEG
    NOC = S // OCH

    cp_mod0 = pltpu.make_async_copy(wmod_hbm.at[:, pl.ds(0, 2 * D)], wmod_v.at[:, pl.ds(0, 2 * D)], sem_mod.at[0])
    cp_mod1 = pltpu.make_async_copy(wmod_hbm.at[:, pl.ds(2 * D, 4 * D)], wmod_v.at[:, pl.ds(2 * D, 4 * D)], sem_mod.at[1])
    cp_x0 = pltpu.make_async_copy(x_hbm.at[pl.ds(0, X0)], xb.at[pl.ds(0, X0)], sem_x.at[0])
    cp_x1 = pltpu.make_async_copy(x_hbm.at[pl.ds(X0, S - X0)], xb.at[pl.ds(X0, S - X0)], sem_x.at[1])
    srcs = (wq_hbm, wk_hbm, wv_hbm)
    dsts = (wq_p, wk_p, wv_p)

    def startup_cp(n):
        if n < 3 * NCH:
            t, c = divmod(n, NCH)
            return pltpu.make_async_copy(srcs[t].at[pl.ds(c * DCH, DCH)], stage.at[n], sem_stage.at[n])
        j = n - 3 * NCH
        return pltpu.make_async_copy(wo_hbm.at[pl.ds(j * WOH, WOH)], wo_v.at[pl.ds(j * WOH, WOH)], sem_wo.at[j])

    NST = 3 * NCH + NWO
    WINDOW = 4

    def ffn_cps():
        cps = []
        for j in range(F // 128):
            cps.append(pltpu.make_async_copy(wg_hbm.at[:, pl.ds(j * 128, 128)], wg_v.at[j], sem_ffn.at[0]))
            cps.append(pltpu.make_async_copy(wu_hbm.at[:, pl.ds(j * 128, 128)], wu_v.at[j], sem_ffn.at[0]))
        for j in range(D // 128):
            cps.append(pltpu.make_async_copy(wd_hbm.at[:, pl.ds(j * 128, 128)], wd_v.at[j], sem_ffn.at[0]))
        return cps

    def out_cp(j):
        return pltpu.make_async_copy(ob.at[pl.ds(j * OCH, OCH)], out_hbm.at[pl.ds(j * OCH, OCH)], sem_out.at[j])

    cp_mod0.start()
    cp_x0.start()
    for n in range(WINDOW):
        startup_cp(n).start()

    cv = jnp.broadcast_to(c_ref[...].astype(F32), (8, D))
    sc = _rnd(cv * jax.nn.sigmoid(cv))
    mod_s[:, 2 * D:6 * D] = jnp.zeros((8, 4 * D), F32)
    r_s[...] = jnp.full(r_s.shape, -jnp.inf, F32)
    h_s[0:M, :] = mem0_ref[...].astype(F32)
    cp_mod0.wait()
    mod_s[:, 0:2 * D] = _rnd(_dot(sc, wmod_v[:, 0:2 * D]))

    def staged(n):
        startup_cp(n).wait()
        if n + WINDOW < NST:
            startup_cp(n + WINDOW).start()
        elif n + WINDOW == NST:
            cp_mod1.start()
        if n < 3 * NCH:
            t, c = divmod(n, NCH)
            tr = pltpu.bitcast(jnp.swapaxes(stage[n], 0, 1), jnp.int32)
            for hd in range(H):
                dsts[t][hd // GH, c * DCH // 2:(c + 1) * DCH // 2, (hd % GH) * Dh:(hd % GH + 1) * Dh] = tr[hd]
        else:
            j = n - 3 * NCH
            for hd in range(j * WOH, (j + 1) * WOH):
                wo_p[hd * Dh // 2:(hd + 1) * Dh // 2, :] = pltpu.bitcast(wo_v[hd], jnp.int32)

    for n in range(3 * NCH):
        staged(n)
    cp_x0.wait()

    qi = lax.broadcasted_iota(jnp.int32, (L, L), 0)
    ki = lax.broadcasted_iota(jnp.int32, (L, L), 1)
    mask = (qi < M) | (qi >= ki)
    scale = Dh ** (-0.5)
    wr = wr_ref[...].astype(F32)

    def mods(i):
        return mod_s[0:1, i * D:(i + 1) * D]

    def pre(s):
        r0 = pl.multiple_of(s * SEG, SEG)
        xs = xb[pl.ds(r0, SEG), :].astype(F32)
        h_s[M:L, :] = _rnd(_ln(xs) * (1.0 + mods(1)) + mods(0))

    def norm2(x1):
        return _rnd(_ln(x1) * (1.0 + mods(4)) + mods(3))

    def resid(r0, n):
        xs = xb[pl.ds(r0, n), :].astype(F32)
        return _rnd(xs + _rnd(mods(2) * a_all[pl.ds(r0, n), :].astype(F32)))

    def post(s):
        r0 = pl.multiple_of(s * SEG, SEG)
        x1 = resid(r0, SEG)
        h2 = norm2(x1)
        r = jnp.sum(h2 * wr, axis=-1, keepdims=True)
        lane = lax.broadcasted_iota(jnp.int32, (SEG, 128), 1)
        r_s[...] = jnp.where(lane == s, r, r_s[...])
        ob[pl.ds(r0, SEG), :] = (x1 + _rnd(mods(5) * h2)).astype(BF16)

    def wtile(ref, g):
        return pltpu.bitcast(ref[g], BF16)

    def softmax(sco):
        sco = jnp.where(mask, sco, -1e9 / scale)
        mx = jnp.max(sco, axis=-1, keepdims=True)
        e = jnp.exp2((sco - mx) * (scale * LOG2E))
        den = jnp.sum(e, axis=-1, keepdims=True)
        inv = pl.reciprocal(den, approx=True)
        inv = inv + inv * (1.0 - den * inv)
        return e * inv

    pre(0)

    def step(s, first=False):
        h = h_s[...]
        if not first:
            post(jnp.maximum(s - 2, 0))
        def qk(q, k):
            return [softmax(_dot_nt(q[:, j * Dh:(j + 1) * Dh], k[:, j * Dh:(j + 1) * Dh])) for j in range(GH)]

        def pv(p, v, g):
            for j in range(GH):
                hd = g * GH + j
                o_s[:, hd * Dh:(hd + 1) * Dh] = _dot(p[j], v[:, j * Dh:(j + 1) * Dh])

        ps = []
        q = k = v = None
        for g in range(NG):
            qn = _dot(h, wtile(wq_p, g))
            if g > 0:
                ps.append(qk(q, k))
            kn = _dot(h, wtile(wk_p, g)).astype(BF16)
            q, k = qn, kn
        for g in range(NG):
            vn = _dot(h, wtile(wv_p, g)).astype(BF16)
            if g == 0:
                ps.append(qk(q, k))
            else:
                pv(ps[g - 1], v, g - 1)
            v = vn
        if first:
            for n in range(3 * NCH, NST):
                staged(n)
        acc = _dot(o_s[:, 0:HS * Dh], pltpu.bitcast(wo_p[0:HS * Dh // 2, :], BF16))
        pv(ps[NG - 1], v, NG - 1)
        acc = acc + _dot(o_s[:, HS * Dh:H * Dh], pltpu.bitcast(wo_p[HS * Dh // 2:H * Dh // 2, :], BF16))
        pre(jnp.minimum(s + 1, NSEG - 1))
        acc = acc.astype(BF16)
        h_s[0:M, :] = acc[0:M].astype(F32)
        a_all[pl.ds(pl.multiple_of(s * SEG, SEG), SEG), :] = acc[M:L]
        if first:
            return

        @pl.when(s == 1)
        def _():
            cp_x1.start()
            cp_mod1.wait()
            mod_s[:, 2 * D:6 * D] = _rnd(_dot(sc, wmod_v[:, 2 * D:6 * D]))

        @pl.when(s == 2)
        def _():
            cp_x1.wait()
            for cp in ffn_cps():
                cp.start()

        @pl.when(jnp.logical_and(s > 8, s % 8 == 1))
        def _():
            j = s // 8 - 1
            r0 = pl.multiple_of(j * OCH, OCH)
            pltpu.make_async_copy(ob.at[pl.ds(r0, OCH)], out_hbm.at[pl.ds(r0, OCH)], sem_out.at[j]).start()

    step(0, first=True)
    lax.fori_loop(1, NSEG, lambda s, c: (step(s), c)[1], 0)
    post(NSEG - 2)
    post(NSEG - 1)

    rr = _rnd(r_s[...])
    ids = lax.broadcasted_iota(jnp.int32, (SEG, 128), 1) * SEG + lax.broadcasted_iota(jnp.int32, (SEG, 128), 0)
    valid = ids < S
    m1 = jnp.max(jnp.where(valid, rr, -jnp.inf))
    i1 = jnp.min(jnp.where((rr == m1) & valid, ids, S))
    rest = valid & (ids != i1)
    m2 = jnp.max(jnp.where(rest, rr, -jnp.inf))
    i2 = jnp.min(jnp.where((rr == m2) & rest, ids, S))
    i1 = jnp.clip(i1, 0, S - 1)
    i2 = jnp.clip(i2, 0, S - 1)

    row16 = lax.broadcasted_iota(jnp.int32, (16, D), 0)

    def load_blk(i):
        b0 = pl.multiple_of((i // 16) * 16, 16)
        x1 = resid(b0, 16)
        return b0, x1, norm2(x1), row16 == (i - b0)

    b1, x1a, h2a, sela = load_blk(i1)
    b2, x1c, h2c, selc = load_blk(i2)
    rowa = jnp.sum(jnp.where(sela, h2a, 0.0), axis=0, keepdims=True)
    rowc = jnp.sum(jnp.where(selc, h2c, 0.0), axis=0, keepdims=True)
    rid = lax.broadcasted_iota(jnp.int32, (8, D), 0)
    xsel = jnp.where(rid == 0, rowa, jnp.where(rid == 1, rowc, 0.0))
    for cp in ffn_cps():
        cp.wait()
    g = jnp.concatenate([_dot(xsel, wg_v[j]) for j in range(F // 128)], axis=1)
    u = jnp.concatenate([_dot(xsel, wu_v[j]) for j in range(F // 128)], axis=1)
    g = _rnd(g)
    g = _rnd(g * jax.nn.sigmoid(g))
    gu = _rnd(g * _rnd(u))
    y = _rnd(jnp.concatenate([_dot(gu, wd_v[j]) for j in range(D // 128)], axis=1))
    s1 = _rnd(jax.nn.sigmoid(jnp.full((1, D), m1, F32)))
    s2 = _rnd(jax.nn.sigmoid(jnp.full((1, D), m2, F32)))
    ya = _rnd(y[0:1] * s1)
    yc = _rnd(y[1:2] * s2)
    upa = jnp.where(sela, ya, 0.0) + jnp.where(row16 == (i2 - b1), yc, 0.0)
    upc = jnp.where(selc, yc, 0.0) + jnp.where(row16 == (i1 - b2), ya, 0.0)
    for j in range(NOC - 1):
        out_cp(j).wait()
    ob[pl.ds(b1, 16), :] = (x1a + _rnd(mods(5) * _rnd(h2a + upa))).astype(BF16)
    ob[pl.ds(b2, 16), :] = (x1c + _rnd(mods(5) * _rnd(h2c + upc))).astype(BF16)
    last0 = (NOC - 1) * OCH
    out_cp(NOC - 1).start()

    def patch_cp(b, k):
        return pltpu.make_async_copy(ob.at[pl.ds(b, 16)], out_hbm.at[pl.ds(b, 16)], sem_patch.at[k])

    send1 = b1 < last0
    send2 = jnp.logical_and(b2 < last0, b2 != b1)

    @pl.when(send1)
    def _():
        patch_cp(b1, 0).start()

    @pl.when(send2)
    def _():
        patch_cp(b2, 1).start()

    @pl.when(send1)
    def _():
        patch_cp(b1, 0).wait()

    @pl.when(send2)
    def _():
        patch_cp(b2, 1).wait()

    out_cp(NOC - 1).wait()


@functools.partial(jax.jit, static_argnames=("A_seg_len",))
def pallas_adaLN_cond__memory_aug_recurrent_mem_tr__moe_arch_mod__prompt_kernel(
    A_x, A_mem0, A_Wq, A_Wk, A_Wv, A_Wo, A_seg_len, B_x, B_w_r, B_w_gate, B_w_up,
    B_w_down, c, w_mod,
):
    del B_x
    B, S, D = A_x.shape
    assert B == 1
    M = A_mem0.shape[1]
    H, Dh = A_Wq.shape[1], A_Wq.shape[2]
    SEG = int(A_seg_len)
    F = B_w_gate.shape[1]
    NCH = D // 128
    hbm = pl.BlockSpec(memory_space=pl.ANY)
    vm = pl.BlockSpec(memory_space=pltpu.VMEM)
    scratch = [
        pltpu.VMEM((S, D), BF16),
        pltpu.VMEM((D, 6 * D), BF16),
        pltpu.VMEM((3 * NCH, 128, H, Dh), BF16),
        pltpu.VMEM((H // GH, D // 2, GH * Dh), jnp.int32),
        pltpu.VMEM((H // GH, D // 2, GH * Dh), jnp.int32),
        pltpu.VMEM((H // GH, D // 2, GH * Dh), jnp.int32),
        pltpu.VMEM((H, Dh, D), BF16),
        pltpu.VMEM((F // 128, D, 128), BF16),
        pltpu.VMEM((F // 128, D, 128), BF16),
        pltpu.VMEM((D // 128, F, 128), BF16),
        pltpu.VMEM((H * Dh // 2, D), jnp.int32),
        pltpu.VMEM((M + SEG, D), F32),
        pltpu.VMEM((M + SEG, H * Dh), F32),
        pltpu.VMEM((S, D), BF16),
        pltpu.VMEM((SEG, 128), F32),
        pltpu.VMEM((8, 6 * D), F32),
        pltpu.VMEM((S, D), BF16),
        pltpu.SemaphoreType.DMA((2,)),
        pltpu.SemaphoreType.DMA((2,)),
        pltpu.SemaphoreType.DMA((3 * NCH,)),
        pltpu.SemaphoreType.DMA((4,)),
        pltpu.SemaphoreType.DMA((1,)),
        pltpu.SemaphoreType.DMA((S // (8 * SEG),)),
        pltpu.SemaphoreType.DMA((2,)),
    ]
    out = pl.pallas_call(
        functools.partial(_kernel, S=S, D=D, H=H, Dh=Dh, M=M, SEG=SEG, F=F),
        in_specs=[hbm, vm, hbm, hbm, hbm, hbm, vm, hbm, hbm, hbm, vm, hbm],
        out_specs=hbm,
        out_shape=jax.ShapeDtypeStruct((S, D), A_x.dtype),
        scratch_shapes=scratch,
        compiler_params=pltpu.CompilerParams(vmem_limit_bytes=120 * 2**20),
    )(A_x.reshape(S, D), A_mem0.reshape(M, D), A_Wq, A_Wk, A_Wv, A_Wo,
      B_w_r.reshape(1, D), B_w_gate, B_w_up, B_w_down, c, w_mod)
    return out.reshape(B, S, D)
```

```python
import functools

import jax
import jax.numpy as jnp
from jax import lax
import jax.experimental.pallas as pl
import jax.experimental.pallas.tpu as pltpu

F32 = jnp.float32
BF16 = jnp.bfloat16
EPS = 1e-05
GH = 8
HTAIL = 16
RB = 64
LEAD = 128
LOG2E = 1.4426950408889634


def _dot(a, b):
    return lax.dot_general(a, b, (((1,), (0,)), ((), ())), preferred_element_type=F32)


def _dot_nt(a, b):
    return lax.dot_general(a, b, (((1,), (1,)), ((), ())), preferred_element_type=F32)


def _ln(x):
    m = jnp.mean(x, axis=-1, keepdims=True)
    d = x - m
    v = jnp.mean(d * d, axis=-1, keepdims=True)
    return d / jnp.sqrt(v + EPS)


def _rnd(x):
    return x.astype(BF16).astype(F32)


def _kernel(x_hbm, mem0_ref, wq_hbm, wk_hbm, wv_hbm, wo_hbm, wr_ref, wg_hbm, wu_hbm,
            wd_hbm, c_ref, wmod_hbm, out_hbm,
            xb, wmod_v, qr, kr, vr, wq_p, wk_p, wv_p,
            wo_p, hl_s, h_s, o_s, a_all, r_s, mod_s, ob,
            sem_x, sem_mod, sem_stage, sem_wo, sem_ffn, sem_out, sem_patch,
            *, S, D, H, Dh, M, SEG, F):
    NSEG = S // SEG
    L = M + SEG
    NB = LEAD // M
    RING = LEAD + SEG
    NG = H // GH
    HS = H - HTAIL
    NWO = 4
    WOH = H // NWO
    X0 = LEAD + 5 * SEG
    OCH = 8 * SEG
    NOC = S // OCH

    cp_mod0 = pltpu.make_async_copy(wmod_hbm.at[:, pl.ds(0, 2 * D)], wmod_v.at[:, pl.ds(0, 2 * D)], sem_mod.at[0])
    cp_mod1 = pltpu.make_async_copy(wmod_hbm.at[:, pl.ds(2 * D, 4 * D)], wmod_v.at[:, pl.ds(2 * D, 4 * D)], sem_mod.at[1])
    cp_x0 = pltpu.make_async_copy(x_hbm.at[pl.ds(0, X0)], xb.at[pl.ds(0, X0)], sem_x.at[0])
    cp_x1 = pltpu.make_async_copy(x_hbm.at[pl.ds(X0, S - X0)], xb.at[pl.ds(X0, S - X0)], sem_x.at[1])
    rings = (qr, kr, vr)
    srcs = (wq_hbm, wk_hbm, wv_hbm)
    dsts = (wq_p, wk_p, wv_p)

    buf = {}

    def ffn_cps():
        cps = []
        for j in range(F // 128):
            cps.append(pltpu.make_async_copy(wg_hbm.at[:, pl.ds(j * 128, 128)], buf['wg'].at[j], sem_ffn.at[0]))
            cps.append(pltpu.make_async_copy(wu_hbm.at[:, pl.ds(j * 128, 128)], buf['wu'].at[j], sem_ffn.at[0]))
        for j in range(D // 128):
            cps.append(pltpu.make_async_copy(wd_hbm.at[:, pl.ds(j * 128, 128)], buf['wd'].at[j], sem_ffn.at[0]))
        return cps

    def out_cp(j):
        return pltpu.make_async_copy(ob.at[pl.ds(j * OCH, OCH)], out_hbm.at[pl.ds(j * OCH, OCH)], sem_out.at[j])

    def stage_cp(g, t):
        h0 = pl.multiple_of(g * GH, GH)
        return pltpu.make_async_copy(srcs[t].at[:, pl.ds(h0, GH)], buf['stage'].at[t * NG + g], sem_stage.at[t * NG + g])

    def wo_cp(j):
        return pltpu.make_async_copy(wo_hbm.at[pl.ds(j * WOH, WOH)], buf['wo'].at[pl.ds(j * WOH, WOH)], sem_wo.at[j])

    def staged(g, t, other):
        stage_cp(g, t).wait()

        @pl.when(g + 1 < NG)
        def _():
            stage_cp(g + 1, t).start()

        @pl.when(g + 1 == NG)
        def _():
            wo_cp(t).start()
            if t == 2:
                wo_cp(3).start()
                cp_mod1.start()

        for c in range(4):
            tr = pltpu.bitcast(jnp.swapaxes(buf['stage'][t * NG + g, c * (D // 4):(c + 1) * (D // 4)], 0, 1), jnp.int32)
            for j in range(GH):
                dsts[t][g, c * (D // 8):(c + 1) * (D // 8), j * Dh:(j + 1) * Dh] = tr[j]
        for c in range(4):
            other(c)

    def staged_wo(j):
        wo_cp(j).wait()
        for hd in range(j * WOH, (j + 1) * WOH):
            wo_p[hd * Dh // 2:(hd + 1) * Dh // 2, :] = pltpu.bitcast(buf['wo'][hd], jnp.int32)

    def silu_c():
        cv = jnp.broadcast_to(c_ref[...].astype(F32), (8, D))
        return _rnd(cv * jax.nn.sigmoid(cv))

    def mods(i):
        return mod_s[0:1, i * D:(i + 1) * D]

    def wtile(ref, g):
        return pltpu.bitcast(ref[g], BF16)

    def norm1(xs):
        return _ln(xs) * (1.0 + mods(1)) + mods(0)

    qi = lax.broadcasted_iota(jnp.int32, (L, L), 0)
    ki = lax.broadcasted_iota(jnp.int32, (L, L), 1)
    mask = (qi < M) | (qi >= ki)
    scale = Dh ** (-0.5)
    wr = wr_ref[...].astype(F32)

    def first_new(s):
        return jnp.where(s < NB, LEAD + (SEG - M) * s, SEG * s)

    def pre(s):
        t0 = first_new(s)
        a0 = pl.multiple_of((t0 // 16) * 16, 16)
        xw = xb[pl.ds(a0, SEG + 16), :].astype(F32)
        xs = jnp.where(t0 == a0, xw[0:SEG], xw[8:SEG + 8])
        h_s[M:L, :] = _rnd(norm1(xs))

    def norm2(x1):
        return _rnd(_ln(x1) * (1.0 + mods(4)) + mods(3))

    def resid(r0, n):
        xs = xb[pl.ds(r0, n), :].astype(F32)
        return _rnd(xs + _rnd(mods(2) * a_all[pl.ds(r0, n), :].astype(F32)))

    def post(s):
        r0 = pl.multiple_of(s * SEG, SEG)
        x1 = resid(r0, SEG)
        h2 = norm2(x1)
        r = jnp.sum(h2 * wr, axis=-1, keepdims=True)
        lane = lax.broadcasted_iota(jnp.int32, (SEG, 128), 1)
        r_s[...] = jnp.where(lane == s, r, r_s[...])
        ob[pl.ds(r0, SEG), :] = (x1 + _rnd(mods(5) * h2)).astype(BF16)

    def softmax(sco):
        sco = jnp.where(mask, sco, -1e9 / scale)
        mx = jnp.max(sco, axis=-1, keepdims=True)
        e = jnp.exp2((sco - mx) * (scale * LOG2E))
        den = jnp.sum(e, axis=-1, keepdims=True)
        inv = pl.reciprocal(den, approx=True)
        inv = inv + inv * (1.0 - den * inv)
        return e * inv

    def step(s, lead, first=False):
        nt = SEG - M if lead else SEG
        h = h_s[0:M + nt, :]

        def project(t, g):
            y = _dot(h, wtile(dsts[t], g))
            if not lead:
                return y
            cols = slice(g * GH * Dh, (g + 1) * GH * Dh)
            t0 = LEAD + nt * s
            for i in range(nt // 8):
                w0 = pl.multiple_of(lax.rem(t0 + 8 * i, RING), 8)
                rings[t][pl.ds(w0, 8), cols] = y[M + 8 * i:M + 8 * (i + 1)]
            r0 = pl.multiple_of(lax.rem(s * SEG, RING), SEG)
            return jnp.concatenate([y[0:M], rings[t][pl.ds(r0, SEG), cols]], axis=0)

        if not first:
            post(jnp.maximum(s - 3, 0))
        def qk(q, k):
            return [softmax(_dot_nt(q[:, j * Dh:(j + 1) * Dh], k[:, j * Dh:(j + 1) * Dh])) for j in range(GH)]

        def pv(p, v, g):
            for j in range(GH):
                hd = g * GH + j
                o_s[:, hd * Dh:(hd + 1) * Dh] = _dot(p[j], v[:, j * Dh:(j + 1) * Dh])

        ps = []
        q = k = v = None
        for g in range(NG):
            qn = project(0, g)
            if g > 0:
                ps.append(qk(q, k))
            kn = project(1, g).astype(BF16)
            q, k = qn, kn
        for g in range(NG):
            vn = project(2, g).astype(BF16)
            if g == 0:
                ps.append(qk(q, k))
            else:
                pv(ps[g - 1], v, g - 1)
            v = vn
        if first:
            for j in range(NWO):
                staged_wo(j)
        acc = _dot(o_s[:, 0:HS * Dh], pltpu.bitcast(wo_p[0:HS * Dh // 2, :], BF16))
        pv(ps[NG - 1], v, NG - 1)
        acc = acc + _dot(o_s[:, HS * Dh:H * Dh], pltpu.bitcast(wo_p[HS * Dh // 2:H * Dh // 2, :], BF16))
        pre(jnp.minimum(s + 1, NSEG - 1))
        acc = acc.astype(BF16)
        h_s[0:M, :] = acc[0:M].astype(F32)
        a_all[pl.ds(pl.multiple_of(s * SEG, SEG), SEG), :] = acc[M:L]
        if first:
            return

        @pl.when(jnp.logical_and(lead, s == 2))
        def _():
            cp_x1.start()
            cp_mod1.wait()
            mod_s[:, 2 * D:6 * D] = _rnd(_dot(silu_c(), wmod_v[:, 2 * D:6 * D]))

        @pl.when(jnp.logical_and(lead, s == 3))
        def _():
            cp_x1.wait()
            for cp in ffn_cps():
                cp.start()

        @pl.when(jnp.logical_and(s > 8, s % 8 == 2))
        def _():
            j = s // 8 - 1
            r0 = pl.multiple_of(j * OCH, OCH)
            pltpu.make_async_copy(ob.at[pl.ds(r0, OCH)], out_hbm.at[pl.ds(r0, OCH)], sem_out.at[j]).start()

    def phase1(stage, wo_v):
        buf.update(stage=stage, wo=wo_v)
        stage_cp(0, 0).start()
        cp_mod0.start()
        cp_x0.start()
        stage_cp(0, 1).start()
        stage_cp(0, 2).start()

        sc = silu_c()
        mod_s[:, 2 * D:6 * D] = jnp.zeros((8, 4 * D), F32)
        r_s[...] = jnp.full(r_s.shape, -jnp.inf, F32)
        h_s[0:M, :] = mem0_ref[...].astype(F32)
        staged(0, 0, lambda c: None)
        cp_mod0.wait()
        mod_s[:, 0:2 * D] = _rnd(_dot(sc, wmod_v[:, 0:2 * D]))

        xb[S:S + 16, :] = jnp.zeros((16, D), BF16)
        cp_x0.wait()
        hl_s[...] = norm1(xb[0:LEAD, :].astype(F32)).astype(BF16)
        BW = GH * Dh // 4

        def bulk(t, g, c):
            c0 = pl.multiple_of(g * GH * Dh + c * BW, BW)
            w = pltpu.bitcast(dsts[t][g, :, c * BW:(c + 1) * BW], BF16)
            for r in range(0, LEAD, RB):
                rings[t][r:r + RB, pl.ds(c0, BW)] = _dot(hl_s[r:r + RB, :], w)


        def group(g, carry):
            staged(g, 1, lambda c: bulk(0, g, c))
            staged(g, 2, lambda c: bulk(1, g, c))

            @pl.when(g + 1 < NG)
            def _():
                staged(g + 1, 0, lambda c: bulk(2, g, c))

            @pl.when(g + 1 == NG)
            def _():
                for c in range(4):
                    bulk(2, g, c)
            return carry

        lax.fori_loop(0, NG, group, 0)
        pre(0)
        step(0, True, first=True)

    pl.run_scoped(phase1, pltpu.VMEM((3 * NG, D, GH, Dh), BF16), pltpu.VMEM((H, Dh, D), BF16))

    def phase2(wg_v, wu_v, wd_v):
        buf.update(wg=wg_v, wu=wu_v, wd=wd_v)
        lax.fori_loop(1, NB, lambda s, c: (step(s, True), c)[1], 0)
        lax.fori_loop(NB, NSEG, lambda s, c: (step(s, False), c)[1], 0)
        post(NSEG - 3)
        post(NSEG - 2)
        post(NSEG - 1)

        rr = _rnd(r_s[...])
        ids = lax.broadcasted_iota(jnp.int32, (SEG, 128), 1) * SEG + lax.broadcasted_iota(jnp.int32, (SEG, 128), 0)
        valid = ids < S
        m1 = jnp.max(jnp.where(valid, rr, -jnp.inf))
        i1 = jnp.min(jnp.where((rr == m1) & valid, ids, S))
        rest = valid & (ids != i1)
        m2 = jnp.max(jnp.where(rest, rr, -jnp.inf))
        i2 = jnp.min(jnp.where((rr == m2) & rest, ids, S))
        i1 = jnp.clip(i1, 0, S - 1)
        i2 = jnp.clip(i2, 0, S - 1)

        row16 = lax.broadcasted_iota(jnp.int32, (16, D), 0)

        def load_blk(i):
            b0 = pl.multiple_of((i // 16) * 16, 16)
            x1 = resid(b0, 16)
            return b0, x1, norm2(x1), row16 == (i - b0)

        b1, x1a, h2a, sela = load_blk(i1)
        b2, x1c, h2c, selc = load_blk(i2)
        rowa = jnp.sum(jnp.where(sela, h2a, 0.0), axis=0, keepdims=True)
        rowc = jnp.sum(jnp.where(selc, h2c, 0.0), axis=0, keepdims=True)
        rid = lax.broadcasted_iota(jnp.int32, (8, D), 0)
        xsel = jnp.where(rid == 0, rowa, jnp.where(rid == 1, rowc, 0.0))
        for cp in ffn_cps():
            cp.wait()
        g = jnp.concatenate([_dot(xsel, buf['wg'][j]) for j in range(F // 128)], axis=1)
        u = jnp.concatenate([_dot(xsel, buf['wu'][j]) for j in range(F // 128)], axis=1)
        g = _rnd(g)
        g = _rnd(g * jax.nn.sigmoid(g))
        gu = _rnd(g * _rnd(u))
        y = _rnd(jnp.concatenate([_dot(gu, buf['wd'][j]) for j in range(D // 128)], axis=1))
        s1 = _rnd(jax.nn.sigmoid(jnp.full((1, D), m1, F32)))
        s2 = _rnd(jax.nn.sigmoid(jnp.full((1, D), m2, F32)))
        ya = _rnd(y[0:1] * s1)
        yc = _rnd(y[1:2] * s2)
        upa = jnp.where(sela, ya, 0.0) + jnp.where(row16 == (i2 - b1), yc, 0.0)
        upc = jnp.where(selc, yc, 0.0) + jnp.where(row16 == (i1 - b2), ya, 0.0)
        for j in range(NOC - 1):
            out_cp(j).wait()
        ob[pl.ds(b1, 16), :] = (x1a + _rnd(mods(5) * _rnd(h2a + upa))).astype(BF16)
        ob[pl.ds(b2, 16), :] = (x1c + _rnd(mods(5) * _rnd(h2c + upc))).astype(BF16)
        last0 = (NOC - 1) * OCH
        out_cp(NOC - 1).start()

        def patch_cp(b, k):
            return pltpu.make_async_copy(ob.at[pl.ds(b, 16)], out_hbm.at[pl.ds(b, 16)], sem_patch.at[k])

        send1 = b1 < last0
        send2 = jnp.logical_and(b2 < last0, b2 != b1)

        @pl.when(send1)
        def _():
            patch_cp(b1, 0).start()

        @pl.when(send2)
        def _():
            patch_cp(b2, 1).start()

        @pl.when(send1)
        def _():
            patch_cp(b1, 0).wait()

        @pl.when(send2)
        def _():
            patch_cp(b2, 1).wait()

        out_cp(NOC - 1).wait()

    pl.run_scoped(phase2, pltpu.VMEM((F // 128, D, 128), BF16), pltpu.VMEM((F // 128, D, 128), BF16),
                  pltpu.VMEM((D // 128, F, 128), BF16))


@functools.partial(jax.jit, static_argnames=("A_seg_len",))
def pallas_adaLN_cond__memory_aug_recurrent_mem_tr__moe_arch_mod__prompt_kernel(
    A_x, A_mem0, A_Wq, A_Wk, A_Wv, A_Wo, A_seg_len, B_x, B_w_r, B_w_gate, B_w_up,
    B_w_down, c, w_mod,
):
    del B_x
    B, S, D = A_x.shape
    assert B == 1
    M = A_mem0.shape[1]
    H, Dh = A_Wq.shape[1], A_Wq.shape[2]
    SEG = int(A_seg_len)
    F = B_w_gate.shape[1]
    hbm = pl.BlockSpec(memory_space=pl.ANY)
    vm = pl.BlockSpec(memory_space=pltpu.VMEM)
    scratch = [
        pltpu.VMEM((S + 16, D), BF16),
        pltpu.VMEM((D, 6 * D), BF16),
        pltpu.VMEM((LEAD + SEG, H * Dh), F32),
        pltpu.VMEM((LEAD + SEG, H * Dh), F32),
        pltpu.VMEM((LEAD + SEG, H * Dh), F32),
        pltpu.VMEM((H // GH, D // 2, GH * Dh), jnp.int32),
        pltpu.VMEM((H // GH, D // 2, GH * Dh), jnp.int32),
        pltpu.VMEM((H // GH, D // 2, GH * Dh), jnp.int32),
        pltpu.VMEM((H * Dh // 2, D), jnp.int32),
        pltpu.VMEM((LEAD, D), BF16),
        pltpu.VMEM((M + SEG, D), F32),
        pltpu.VMEM((M + SEG, H * Dh), F32),
        pltpu.VMEM((S, D), BF16),
        pltpu.VMEM((SEG, 128), F32),
        pltpu.VMEM((8, 6 * D), F32),
        pltpu.VMEM((S, D), BF16),
        pltpu.SemaphoreType.DMA((2,)),
        pltpu.SemaphoreType.DMA((2,)),
        pltpu.SemaphoreType.DMA((3 * (H // GH),)),
        pltpu.SemaphoreType.DMA((4,)),
        pltpu.SemaphoreType.DMA((1,)),
        pltpu.SemaphoreType.DMA((S // (8 * SEG),)),
        pltpu.SemaphoreType.DMA((2,)),
    ]
    out = pl.pallas_call(
        functools.partial(_kernel, S=S, D=D, H=H, Dh=Dh, M=M, SEG=SEG, F=F),
        in_specs=[hbm, vm, hbm, hbm, hbm, hbm, vm, hbm, hbm, hbm, vm, hbm],
        out_specs=hbm,
        out_shape=jax.ShapeDtypeStruct((S, D), A_x.dtype),
        scratch_shapes=scratch,
        compiler_params=pltpu.CompilerParams(vmem_limit_bytes=126 * 2**20),
    )(A_x.reshape(S, D), A_mem0.reshape(M, D), A_Wq, A_Wk, A_Wv, A_Wo,
      B_w_r.reshape(1, D), B_w_gate, B_w_up, B_w_down, c, w_mod)
    return out.reshape(B, S, D)
```
